```python
import os as _os
_os.environ.setdefault("JAX_PLATFORMS", "cpu")
import jax
import jax.numpy as jnp

def _softmax(x, axis=-1):
    return jax.nn.softmax(x, axis=axis)
def _gelu(x):
    return jax.nn.gelu(x, approximate=True)
def _silu(x):
    return jax.nn.silu(x)
def _sigmoid(x):
    return jax.nn.sigmoid(x)
def _layernorm(x, axis=-1, eps=1e-5):
    m = jnp.mean(x, axis=axis, keepdims=True)
    v = jnp.var(x, axis=axis, keepdims=True)
    return (x - m) / jnp.sqrt(v + eps)
def _scatter_add(tgt, idx, src, axis=0):
    return tgt.at[idx].add(src)
def _segment_sum(src, seg, n):
    return jax.ops.segment_sum(src, seg, n)
class _Rng:
    def __init__(self, key):
        self._k = key
    def _next(self):
        self._k, sub = jax.random.split(self._k)
        return sub
    def normal(self, shape):
        return jax.random.normal(self._next(), shape, dtype=jnp.bfloat16)
    def randint(self, lo, hi, shape):
        return jax.random.randint(self._next(), shape, lo, hi, dtype=jnp.int32)
    def uniform(self, shape, lo=0.0, hi=1.0):
        return jax.random.uniform(self._next(), shape, jnp.bfloat16, lo, hi)
    def permutation(self, n):
        return jax.random.permutation(self._next(), n)


kernel_name = 'sequential_preLN__spectral_gfnet__glu_gated_bilinear__prompt'

def setup_inputs():
    _rng = _Rng(jax.random.key(int.from_bytes(__import__("os").urandom(4), "little")))
    _w = (lambda a: (lambda t: t.astype(jnp.bfloat16) if jnp.issubdtype(t.dtype, jnp.floating) else t)(jnp.asarray(a)))
    def _A_setup():
        B, S, D = 1, 2048, 448
        Df = D // 2 + 1
        return {
            "x": _w((lambda *s: _rng.normal(s) * 0.05)(B, S, D)),
            "w_r": _w((lambda *s: _rng.normal(s) * 0.2)(S, Df) * 0.02),
            "w_i": _w((lambda *s: _rng.normal(s) * 0.2)(S, Df) * 0.02),
        }
    _A_in = _A_setup()

    def _B_setup():
        B, S, D, F = 1, 2048, 448, 1792
        return {
            "x": _w((lambda *s: _rng.normal(s) * 0.05)(B, S, D)),
            "w_gate": _w((lambda *s: _rng.normal(s) * 0.05)(D, F) * (D ** -0.5)),
            "w_up": _w((lambda *s: _rng.normal(s) * 0.05)(D, F) * (D ** -0.5)),
            "w_down": _w((lambda *s: _rng.normal(s) * 0.05)(F, D) * (F ** -0.5)),
        }
    _B_in = _B_setup()

    return {
        "A_x": _A_in["x"],
        "A_w_r": _A_in["w_r"],
        "A_w_i": _A_in["w_i"],
        "B_x": _B_in["x"],
        "B_w_gate": _B_in["w_gate"],
        "B_w_up": _B_in["w_up"],
        "B_w_down": _B_in["w_down"],
    }

def reference(A_x, A_w_r, A_w_i, B_x, B_w_gate, B_w_up, B_w_down):
    def _A_ref(x, w_r, w_i):
        B, S, D = x.shape
        X = (lambda x, axes=(-2,-1): jnp.fft.rfft2(x.astype(jnp.float32), axes=axes))(x, axes=(-2, -1))
        W = w_r + 1j * w_i
        X = X * W
        y = (lambda x, s, axes=(-2,-1): jnp.fft.irfft2(x, s=s, axes=axes).astype(jnp.bfloat16))(X, (S, D), axes=(-2, -1))
        return y

    def _B_ref(x, w_gate, w_up, w_down):
        g = jnp.einsum("bsd,df->bsf", x, w_gate)
        u = jnp.einsum("bsd,df->bsf", x, w_up)
        h = g * u
        return jnp.einsum("bsf,fd->bsd", h, w_down)

    x = A_x
    h = x + _A_ref(_layernorm(x, axis=-1), A_w_r, A_w_i)
    h2 = h + _B_ref(_layernorm(h, axis=-1), B_w_gate, B_w_up, B_w_down)
    return h2
```

```python
import functools
import numpy as np
import jax
import jax.numpy as jnp
from jax.experimental import pallas as pl
from jax.experimental.pallas import tpu as pltpu

S, D, F = 2048, 448, 1792
H = D // 2
NT = S // 128
BF = jnp.bfloat16
F32 = jnp.float32


def _np_bf16(a):
    return np.asarray(a, np.float32).astype(jnp.bfloat16.dtype)


def _interleave_rows(a, b):
    n = a.shape[1]
    return np.stack([a.reshape(H // 8, 8, n), b.reshape(H // 8, 8, n)], axis=1).reshape(2 * H, n)


def _consts():
    jslot = np.arange(H); jslot[0] = H
    d = np.arange(D)
    ang = 2 * np.pi * np.outer(jslot, d) / D
    fr = np.cos(ang); fi = -np.sin(ang); fi[0] = 0
    rf = _interleave_rows(fr, fi)
    c = np.full(H, 2.0); c[0] = 1.0
    gr = np.cos(ang) * c[:, None] / (S * D)
    gi = -np.sin(ang) * c[:, None] / (S * D); gi[0] = 0
    ri = _interleave_rows(gr, gi).T
    lane = np.arange(128)
    k1 = 8 * (lane & 15) + (lane >> 4)
    mm = []
    for k2 in range(16):
        m = np.exp(-2j * np.pi * np.outer(np.arange(128), k2 + 16 * k1) / S)
        mm.append(np.concatenate([m.real, m.imag], axis=1))
    return _np_bf16(rf), _np_bf16(ri), _np_bf16(np.stack(mm))


_RF, _RI, _MM = _consts()


def _dft4(a, sign):
    (r0, i0), (r1, i1), (r2, i2), (r3, i3) = a
    ar, ai = r0 + r2, i0 + i2
    br, bi = r0 - r2, i0 - i2
    cr, ci = r1 + r3, i1 + i3
    dr, di = r1 - r3, i1 - i3
    y0 = (ar + cr, ai + ci)
    y2 = (ar - cr, ai - ci)
    if sign < 0:
        y1 = (br + di, bi - dr)
        y3 = (br - di, bi + dr)
    else:
        y1 = (br - di, bi + dr)
        y3 = (br + di, bi - dr)
    return [y0, y1, y2, y3]


def _tw(v, n, sign):
    n = n % 16
    r, i = v
    if n == 0:
        return v
    if n == 4:
        return (i, -r) if sign < 0 else (-i, r)
    if n == 8:
        return (-r, -i)
    if n == 12:
        return (-i, r) if sign < 0 else (i, -r)
    c = float(np.cos(2 * np.pi * n / 16)); s = float(sign * np.sin(2 * np.pi * n / 16))
    if n % 2 == 0:
        sc, ss = np.sign(c), np.sign(s)
        h = abs(c)
        t1 = (r - i) if sc * ss > 0 else (r + i)
        t2 = (i + r) if sc * ss > 0 else (i - r)
        return (t1 * (h * sc), t2 * (h * sc))
    return (r * c - i * s, r * s + i * c)


def _dft16(v, sign):
    cols = [_dft4([v[n2 + 4 * n1] for n1 in range(4)], sign) for n2 in range(4)]
    out = [None] * 16
    for k1 in range(4):
        y = _dft4([_tw(cols[n2][k1], n2 * k1, sign) for n2 in range(4)], sign)
        for k2 in range(4):
            out[k1 + 4 * k2] = y[k2]
    return out


def _ln_rows(xf):
    m = jnp.mean(xf, axis=0, keepdims=True)
    xc = xf - m
    v = jnp.mean(xc * xc, axis=0, keepdims=True)
    return xc * jax.lax.rsqrt(v + 1e-5)


def _kernel(xT_h, wr_h, wi_h, wg_h, wu_h, wd_h, rf_h, ri_h, mm_h, out_h,
            x_v, wr_v, wi_v, wg_v, wu_v, wd_v, rf_v, ri_v, mm_v,
            wgT_v, wuT_v, z_v, u_v, wsr_v, wsi_v, yd_v, h_v, ln_v, o_v, sem, osem,
            *, tb, tm):
    nxb = S // tb
    xcp = [pltpu.make_async_copy(xT_h.at[:, pl.ds(b * tb, tb)], x_v.at[:, pl.ds(b * tb, tb)], sem.at[b])
           for b in range(nxb)]
    others = [(rf_h, rf_v), (wr_h, wr_v), (wi_h, wi_v), (mm_h, mm_v), (ri_h, ri_v),
              (wg_h, wg_v), (wu_h, wu_v), (wd_h, wd_v)]
    cp = [pltpu.make_async_copy(a, b, sem.at[nxb + i]) for i, (a, b) in enumerate(others)]
    c_rf, c_wr, c_wi, c_mm, c_ri, c_wg, c_wu, c_wd = cp
    xcp[0].start()
    c_rf.start()
    for c in xcp[1:]:
        c.start()
    for c in cp[1:]:
        c.start()

    c_rf.wait()
    for b in range(nxb):
        xcp[b].wait()
        lo = b * tb
        ln = _ln_rows(x_v[:, lo:lo + tb].astype(F32)).astype(BF)
        z_v[:, lo:lo + tb] = jnp.dot(rf_v[...], ln, preferred_element_type=F32)

    for g in range(H // 8):
        v = [(z_v[16 * g:16 * g + 8, 128 * t:128 * t + 128], z_v[16 * g + 8:16 * g + 16, 128 * t:128 * t + 128])
             for t in range(NT)]
        o = _dft16(v, -1)
        for k2 in range(16):
            u_v[k2, 16 * g:16 * g + 16, :] = jnp.concatenate(o[k2], axis=0).astype(BF)

    c_wr.wait(); c_wi.wait()
    lane = jax.lax.broadcasted_iota(jnp.int32, (8, 128), 1)
    for w_v, ws_v in ((wr_v, wsr_v), (wi_v, wsi_v)):
        for G in range(H // 16):
            T = []
            for t in range(NT):
                blk = w_v[16 * G:16 * G + 16, 128 * t:128 * t + 128]
                if G == 0:
                    row = jax.lax.broadcasted_iota(jnp.int32, (16, 128), 0)
                    last = w_v[H:H + 1, 128 * t:128 * t + 128].astype(F32)
                    blk = jnp.where(row == 0, last, blk.astype(F32)).astype(BF)
                T.append(pltpu.bitcast(blk, jnp.int32))
            for i in range(4):
                dl = 1 << i
                m0 = (lane & dl) == 0
                for t in range(NT):
                    if t & dl:
                        continue
                    a, b = T[t], T[t | dl]
                    T[t] = jnp.where(m0, a, pltpu.roll(b, dl, 1))
                    T[t | dl] = jnp.where(m0, pltpu.roll(a, 128 - dl, 1), b)
            for t in range(NT):
                ws_v[t, 16 * G:16 * G + 16, :] = pltpu.bitcast(T[t], BF)

    c_mm.wait()
    for k2 in range(16):
        mmk = mm_v[k2]
        ab = jnp.dot(u_v[k2], mmk, preferred_element_type=F32).reshape(H // 8, 16, 256)
        xr = ab[:, :8, :128] - ab[:, 8:, 128:]
        xi = ab[:, :8, 128:] + ab[:, 8:, :128]
        wr = wsr_v[k2].astype(F32).reshape(H // 8, 8, 128)
        wi = wsi_v[k2].astype(F32).reshape(H // 8, 8, 128)
        vr = xr * wr - xi * wi
        vi = xr * wi + xi * wr
        l2 = jnp.concatenate([vr, vi], axis=1).reshape(2 * H, 128).astype(BF)
        nt = (((1,), (1,)), ((), ()))
        a2 = jax.lax.dot_general(l2, mmk[:, :128], nt, preferred_element_type=F32).reshape(H // 8, 16, 128)
        b2 = jax.lax.dot_general(l2, mmk[:, 128:], nt, preferred_element_type=F32).reshape(H // 8, 16, 128)
        pr = a2[:, :8] + b2[:, 8:]
        pi = a2[:, 8:] - b2[:, :8]
        z_v[:, 128 * k2:128 * k2 + 128] = jnp.concatenate([pr, pi], axis=1).reshape(2 * H, 128)

    for g in range(H // 8):
        v = [(z_v[16 * g:16 * g + 8, 128 * t:128 * t + 128], z_v[16 * g + 8:16 * g + 16, 128 * t:128 * t + 128])
             for t in range(NT)]
        o = _dft16(v, +1)
        for t in range(16):
            yd_v[16 * g:16 * g + 16, 128 * t:128 * t + 128] = jnp.concatenate(o[t], axis=0).astype(BF)

    c_ri.wait(); c_wg.wait(); c_wu.wait(); c_wd.wait()
    for c in range(F // 128):
        wgT_v[128 * c:128 * c + 128, :] = wg_v[:, 128 * c:128 * c + 128].T
        wuT_v[128 * c:128 * c + 128, :] = wu_v[:, 128 * c:128 * c + 128].T

    nb = S // tm

    def ocp(b):
        return pltpu.make_async_copy(o_v.at[b % 2], out_h.at[:, pl.ds(pl.multiple_of(b * tm, tm), tm)], osem.at[b % 2])

    def body(b, carry):
        lo = pl.multiple_of(b * tm, tm)
        y = jnp.dot(ri_v[...], yd_v[:, pl.ds(lo, tm)], preferred_element_type=F32)
        h = x_v[:, pl.ds(lo, tm)].astype(F32) + y
        ln = _ln_rows(h).astype(BF)
        g = jnp.dot(wgT_v[...], ln, preferred_element_type=F32)
        u = jnp.dot(wuT_v[...], ln, preferred_element_type=F32)
        hh = (g * u).astype(BF)
        o = jnp.dot(wd_v[...], hh, preferred_element_type=F32)

        @pl.when(b >= 2)
        def _():
            ocp(b - 2).wait()
        o_v[b % 2] = (h + o).astype(BF)
        ocp(b).start()
        return carry

    jax.lax.fori_loop(0, nb, body, 0)
    ocp(nb - 2).wait()
    ocp(nb - 1).wait()


def make(tb=512, tm=512):
    @jax.jit
    def f(A_x, A_w_r, A_w_i, B_x, B_w_gate, B_w_up, B_w_down):
        del B_x
        xT = A_x.reshape(S, D).T
        anyspec = pl.BlockSpec(memory_space=pl.ANY)
        scratch = [
            pltpu.VMEM((D, S), BF), pltpu.VMEM((H + 1, S), BF), pltpu.VMEM((H + 1, S), BF),
            pltpu.VMEM((D, F), BF), pltpu.VMEM((D, F), BF), pltpu.VMEM((D, F), BF),
            pltpu.VMEM((D, D), BF), pltpu.VMEM((D, D), BF), pltpu.VMEM((16, 128, 256), BF),
            pltpu.VMEM((F, D), BF), pltpu.VMEM((F, D), BF),
            pltpu.VMEM((D, S), F32), pltpu.VMEM((16, D, 128), BF),
            pltpu.VMEM((16, H, 128), BF), pltpu.VMEM((16, H, 128), BF),
            pltpu.VMEM((D, S), BF), pltpu.VMEM((8, 128), F32), pltpu.VMEM((8, 128), BF),
            pltpu.VMEM((2, D, tm), BF),
            pltpu.SemaphoreType.DMA((S // tb + 8,)), pltpu.SemaphoreType.DMA((2,)),
        ]
        outT = pl.pallas_call(
            functools.partial(_kernel, tb=tb, tm=tm),
            in_specs=[anyspec] * 9, out_specs=anyspec,
            out_shape=jax.ShapeDtypeStruct((D, S), BF),
            scratch_shapes=scratch,
            compiler_params=pltpu.CompilerParams(vmem_limit_bytes=100 * 1024 * 1024),
        )(xT, A_w_r.T, A_w_i.T, B_w_gate, B_w_up, B_w_down.T, _RF, _RI, _MM)
        return outT.T.reshape(1, S, D)
    return f


_fn = make()


def pallas_sequential_preLN__spectral_gfnet__glu_gated_bilinear__prompt_kernel(A_x, A_w_r, A_w_i, B_x, B_w_gate, B_w_up, B_w_down):
    return _fn(A_x, A_w_r, A_w_i, B_x, B_w_gate, B_w_up, B_w_down)
```

```python
import contextlib
import functools
import numpy as np
import jax
import jax.numpy as jnp
from jax.experimental import pallas as pl
from jax.experimental.pallas import tpu as pltpu

S, D, F = 2048, 448, 1792
H = D // 2
NT = S // 128
NG = H // 8
BF = jnp.bfloat16
F32 = jnp.float32
I32 = jnp.int32

CLASSES = [[0, 7], [1, 8, 6, 13], [2, 9, 5, 12], [3, 10, 4, 11]]
GROUPS = [(m, kap, qh) for m in range(4) for kap in CLASSES[m] for qh in range(2)]
BLK_OFF = [0, 64, 192, 320, 448]


def _np_bf16(a):
    return np.asarray(a, np.float32).astype(jnp.bfloat16.dtype)


def _np_packed(a):
    u = _np_bf16(a).view(np.uint16).astype(np.uint32)
    return (u[..., 0::2, :] | (u[..., 1::2, :] << 16)).view(np.int32)


def _pk(v):
    return pltpu.bitcast(v.astype(BF), I32)


def _upk(v):
    return pltpu.bitcast(v, BF)


def _group_bins(g):
    _, kap, qh = GROUPS[g]
    j = 14 * (8 * qh + np.arange(8)) + kap
    return np.where(j == 0, H, j)


def _lane_k(k2):
    m = np.arange(128)
    t = ((m & 15) - k2) % 16
    return 128 * t + (m - t) % 128


def _consts():
    b = np.arange(64)
    tf, ti = [], []
    for m in range(4):
        rows, cols = [], []
        for g in [g for g in range(NG) if GROUPS[g][0] == m]:
            j = _group_bins(g)
            th = 2 * np.pi * np.outer(j, b) / D
            c, s = np.cos(th), np.sin(th)
            if m == 0:
                fre, fim = c, np.where((j == H)[:, None], 0.0, -s)
                w = np.where(j == H, 1.0, 2.0)[:, None] / (S * D)
                ivr, ivi = (c * w).T, (fim * w).T
            else:
                sg = np.where((j % 7) == m, 1.0, -1.0)[:, None]

                def kord(p, q):
                    return np.stack([p.reshape(8, 4, 16), q.reshape(8, 4, 16)], axis=2).reshape(8, 128)
                fre, fim = kord(c, -sg * s), kord(-s, -sg * c)
                w = 2.0 / (S * D)
                ivr = np.concatenate([c * w, sg * s * w], 1).T
                ivi = np.concatenate([-s * w, sg * c * w], 1).T
            rows += [fre, fim]
            cols += [ivr, ivi]
        tf.append(np.concatenate(rows, 0))
        ti.append(np.concatenate(cols, 1))
    t0 = np.stack([tf[0], ti[0]])
    tm = np.stack(tf[1:] + ti[1:] + [np.zeros((128, 128))])
    mm = []
    for k2 in range(16):
        e = np.exp(-2j * np.pi * np.outer(np.arange(128), _lane_k(k2)) / S)
        mm.append(np.concatenate([e.real, e.imag], axis=1))
    return _np_packed(t0), _np_packed(tm), _np_packed(np.stack(mm))


_T0, _TM, _MM = _consts()
_C7 = [float(np.cos(2 * np.pi * n / 7)) for n in range(7)]
_S7 = [float(np.sin(2 * np.pi * n / 7)) for n in range(7)]


def _dft4(a, sign):
    (r0, i0), (r1, i1), (r2, i2), (r3, i3) = a
    ar, ai = r0 + r2, i0 + i2
    br, bi = r0 - r2, i0 - i2
    cr, ci = r1 + r3, i1 + i3
    dr, di = r1 - r3, i1 - i3
    y0 = (ar + cr, ai + ci)
    y2 = (ar - cr, ai - ci)
    if sign < 0:
        y1 = (br + di, bi - dr)
        y3 = (br - di, bi + dr)
    else:
        y1 = (br - di, bi + dr)
        y3 = (br + di, bi - dr)
    return [y0, y1, y2, y3]


def _tw(v, n, sign):
    n = n % 16
    r, i = v
    if n == 0:
        return v
    if n == 4:
        return (i, -r) if sign < 0 else (-i, r)
    c = float(np.cos(2 * np.pi * n / 16))
    s = float(sign * np.sin(2 * np.pi * n / 16))
    if n % 2 == 0:
        same = (c * s) > 0
        t1 = (r - i) if same else (r + i)
        t2 = (i + r) if same else (i - r)
        return (t1 * c, t2 * c)
    return (r * c - i * s, r * s + i * c)


def _dft16(v, sign):
    cols = [_dft4([v[n2 + 4 * n1] for n1 in range(4)], sign) for n2 in range(4)]
    out = [None] * 16
    for k1 in range(4):
        y = _dft4([_tw(cols[n2][k1], n2 * k1, sign) for n2 in range(4)], sign)
        for k2 in range(4):
            out[k1 + 4 * k2] = y[k2]
    return out


def _lin(vals, coefs, base=None):
    acc = base
    for v, c in zip(vals, coefs):
        t = v * c
        acc = t if acc is None else acc + t
    return acc


def _ln_rows(xf):
    m = jnp.mean(xf, axis=0, keepdims=True)
    xc = xf - m
    v = jnp.mean(xc * xc, axis=0, keepdims=True)
    return xc * jax.lax.rsqrt(v + 1e-5)


def _kernel(xT_h, wr_h, wi_h, wg_h, wu_h, wd_h, t0_h, tm_h, mm_h, zs_h, out_h,
            x_v, wr_v, wi_v, wg_v, wu_v, wd_v, t0_v, tm_v, mm_v,
            zs_s, ud_l, r_v, m1_v, z_v, u_v, ws_v, yd_l, v_v, h_l, ln_v, hh_v, o_v, sem, osem,
            *, tb, tm, fc, kw0, kw1, lag, scopes, bmode, order, retile, kc, wpos, dn, bar, unroll, tail, opq, tie, tlag, chain, nsp, pbar, peel_last, morder, rows_, wdc, wdmid, fsplit, xch, ra1):
    sc = (lambda n: jax.named_scope(n)) if scopes else (lambda n: contextlib.nullcontext())
    nxb = S // tb
    nfc = F // fc
    sems = iter(range(64))

    def copy(a, b):
        return pltpu.make_async_copy(a, b, sem.at[next(sems)])
    xo = [0]
    for n_ in xch:
        xo.append(xo[-1] + n_)
    assert xo[-1] == NT
    c_x = [copy(xT_h.at[:, pl.ds(128 * xo[b], 128 * xch[b])], x_v.at[:, pl.ds(128 * xo[b], 128 * xch[b])]) for b in range(len(xch))]
    c_t0, c_tm = copy(t0_h, t0_v), copy(tm_h, tm_v)
    c_mm, c_wr, c_wi = copy(mm_h, mm_v), copy(wr_h, wr_v), copy(wi_h, wi_v)
    fh = fsplit * fc
    c_wg = [copy(wg_h.at[:, pl.ds(0, fh)], wg_v.at[:, pl.ds(0, fh)])]
    c_wgb = [copy(wg_h.at[:, pl.ds(fh, F - fh)], wg_v.at[:, pl.ds(fh, F - fh)])] if fh < F else []
    c_wu = [copy(wu_h.at[:, pl.ds(0, fh)], wu_v.at[:, pl.ds(0, fh)])]
    c_wub = [copy(wu_h.at[:, pl.ds(fh, F - fh)], wu_v.at[:, pl.ds(fh, F - fh)])] if fh < F else []
    c_wd = copy(wd_h, wd_v)
    c_zs = copy(zs_h, zs_s)
    c_zs.start()
    c_x[0].start()
    c_t0.start()
    c_tm.start()
    for c in c_x[1:]:
        c.start()
    c_mm.start()
    c_wr.start()
    c_wi.start()
    for c in c_wg + c_wu + c_wgb + c_wub:
        c.start()
    c_wd.start()

    c_zs.wait()
    zero = zs_s[0]

    def ods(start, n):
        return pl.ds(pl.multiple_of(zero + start, 128), n) if opq else pl.ds(start, n)

    rs = {}

    def vpu_fwd(t):
        lo = 128 * t
        ud = ud_l[t % len(ud_l)]; ul = slice(128 * (t // len(ud_l)), 128 * (t // len(ud_l)) + 128)
        u0s = []
        sq = None
        for bg in range(4):
            xa = [x_v[64 * a + 16 * bg:64 * a + 16 * bg + 16, lo:lo + 128].astype(F32) for a in range(7)]
            s_ = [xa[a] + xa[7 - a] for a in (1, 2, 3)]
            d_ = [xa[a] - xa[7 - a] for a in (1, 2, 3)]
            u0s.append(xa[0] + s_[0] + s_[1] + s_[2])
            for m in (1, 2, 3):
                ur = _lin(s_, [_C7[(m * a) % 7] for a in (1, 2, 3)], xa[0])
                ui = _lin(d_, [_S7[(m * a) % 7] for a in (1, 2, 3)])
                ud[64 * m - 32 + 16 * bg:64 * m - 24 + 16 * bg, ul] = _pk(ur)
                ud[64 * m - 24 + 16 * bg:64 * m - 16 + 16 * bg, ul] = _pk(ui)
                q = ur * ur + ui * ui
                sq = q if sq is None else sq + q
        m7 = jnp.sum(u0s[0] + u0s[1] + u0s[2] + u0s[3], axis=0, keepdims=True) * (1.0 / 64)
        sq = sq + sq
        for bg in range(4):
            uc = u0s[bg] - m7
            ud[8 * bg:8 * bg + 8, ul] = _pk(uc)
            sq = sq + uc * uc
        var = jnp.sum(sq, axis=0, keepdims=True) * (1.0 / (7 * D))
        r_v[:, lo:lo + 128] = jnp.broadcast_to(jax.lax.rsqrt(var + 1e-5), (8, 128))
        m1_v[:, lo:lo + 128] = jnp.broadcast_to(m7 * (1.0 / 7), (8, 128))

    def mxu_fwd(t):
        lo = 128 * t

        def rr(n):
            return r_v[0:1, lo:lo + 128] if ra1 else 1.0
        ud = ud_l[t % len(ud_l)]; ul = ods(128 * (t // len(ud_l)), 128) if (opq & 1) else slice(128 * (t // len(ud_l)), 128 * (t // len(ud_l)) + 128)
        z_v[0:64, lo:lo + 128] = jnp.dot(_upk(t0_v[0]), _upk(ud[0:32, ul]), preferred_element_type=F32) * rr(64)
        for m in (1, 2, 3):
            z_v[BLK_OFF[m]:BLK_OFF[m + 1], lo:lo + 128] = \
                jnp.dot(_upk(tm_v[m - 1]), _upk(ud[BLK_OFF[m] // 2:BLK_OFF[m + 1] // 2, ul]), preferred_element_type=F32) * rr(128)

    with sc('A1'):
        for r_ in range(len(xch) + 1):
            if r_ < len(xch):
                with sc('w_x%d' % r_):
                    c_x[r_].wait()
            if r_ == 1:
                c_t0.wait()
                c_tm.wait()
            if r_ > 0:
                for t in range(xo[r_ - 1], xo[r_]):
                    mxu_fwd(t)
            if r_ < len(xch):
                for t in range(xo[r_], xo[r_ + 1]):
                    vpu_fwd(t)

    def dft16_pass(sign, store, after=None, gorder=range(NG)):
        for g in gorder:
            v = [(z_v[16 * g:16 * g + 8, 128 * t:128 * t + 128], z_v[16 * g + 8:16 * g + 16, 128 * t:128 * t + 128])
                 for t in range(NT)]
            if sign < 0 and not ra1:
                v = [(a * r_v[:, 128 * t:128 * t + 128], b_ * r_v[:, 128 * t:128 * t + 128]) for t, (a, b_) in enumerate(v)]
            o = _dft16(v, sign)
            for t in range(16):
                store(g, t, _pk(jnp.concatenate(o[t], axis=0)))
            if after is not None:
                after(g)

    with sc('A2'):
        def st(g, t, val):
            u_v[8 * g:8 * g + 8, 128 * t:128 * t + 128] = val
        dft16_pass(-1, st)

    lane = jax.lax.broadcasted_iota(I32, (8, 128), 1)
    bits = [(lane & (1 << i)) != 0 for i in range(4)]

    def scramble(a, G):
        w_v = (wr_v, wi_v)[a]
        cur = []
        for t in range(NT):
            blk = w_v[16 * G:16 * G + 16, 128 * t:128 * t + 128]
            if G == 0:
                row = jax.lax.broadcasted_iota(I32, (16, 128), 0)
                last = w_v[H:H + 1, 128 * t:128 * t + 128].astype(F32)
                blk = jnp.where(row == 0, last, blk.astype(F32)).astype(BF)
            v = pltpu.bitcast(blk, I32)
            cur.append(pltpu.roll(v, t, 1) if t else v)
        for i in range(4):
            cur = [jnp.where(bits[i], cur[(v + (1 << i)) % NT], cur[v]) for v in range(NT)]
        for k2 in range(NT):
            ws_v[a, k2, 8 * G:8 * G + 8, :] = cur[(-k2) % NT]

    def wload(a, k2):
        cls = [None] * 14
        for c in range(7):
            w = ws_v[a, k2, pl.ds(c, 16, stride=7), :]
            cls[2 * c] = pltpu.bitcast(w << 16, F32)
            cls[2 * c + 1] = pltpu.bitcast(w & jnp.int32(-65536), F32)
        return jnp.concatenate([cls[kap] for m in range(4) for kap in CLASSES[m]], axis=0).reshape(NG, 8, 128)

    NGG = H // 16
    with sc('A3a'):
        with sc('w_mm'):
            c_mm.wait()
        todo = [(a, G) for G in range(NGG) for a in range(2)]
        for k2 in range(16):
            if k2 == kw0:
                with sc('w_wr'):
                    c_wr.wait()
                with sc('w_wi'):
                    c_wi.wait()
            ab = jnp.dot(_upk(u_v[:, 128 * k2:128 * k2 + 128]), _upk(mm_v[k2]), preferred_element_type=F32).reshape(NG, 16, 256)
            xr = ab[:, :8, :128] - ab[:, 8:, 128:]
            xi = ab[:, :8, 128:] + ab[:, 8:, :128]
            z_v[:, 128 * k2:128 * k2 + 128] = jnp.concatenate([xr, xi], axis=1).reshape(2 * H, 128)
            if k2 >= kw0:
                n = -(-len(todo) // (16 - k2))
                for _ in range(n):
                    scramble(*todo.pop(0))

    with sc('A3b'):
        nt = (((1,), (1,)), ((), ()))
        for k2 in range(16):
            mmk = _upk(mm_v[k2])
            xx = z_v[:, 128 * k2:128 * k2 + 128].reshape(NG, 16, 128)
            xr, xi = xx[:, :8], xx[:, 8:]
            wr = wload(0, k2)
            wi = wload(1, k2)
            vr = xr * wr - xi * wi
            vi = xr * wi + xi * wr
            l2 = jnp.concatenate([vr, vi], axis=1).reshape(2 * H, 128).astype(BF)
            a2 = jax.lax.dot_general(l2, mmk[:, :128], nt, preferred_element_type=F32).reshape(NG, 16, 128)
            b2 = jax.lax.dot_general(l2, mmk[:, 128:], nt, preferred_element_type=F32).reshape(NG, 16, 128)
            pr = a2[:, :8] + b2[:, 8:]
            pi = a2[:, 8:] - b2[:, :8]
            z_v[:, 128 * k2:128 * k2 + 128] = jnp.concatenate([pr, pi], axis=1).reshape(2 * H, 128)

    with sc('A4'):
        def st(g, t, val):
            m = GROUPS[g][0]
            gg = g - BLK_OFF[m] // 16
            yd_l[m][8 * gg:8 * gg + 8, 128 * t:128 * t + 128] = val

        def inv_d(m):
            tmat = _upk(t0_v[1]) if m == 0 else _upk(tm_v[2 + m])
            for c in range(S // dn):
                ls = slice(c * dn, (c + 1) * dn)
                lr = ods(c * dn, dn) if (opq & 2) else ls
                v_v[BLK_OFF[m]:BLK_OFF[m + 1], ls] = jnp.dot(
                    tmat, _upk(yd_l[m][:, lr]), preferred_element_type=F32)

        def after(g):
            for m in range(4):
                if 16 * (g + 1) == BLK_OFF[m + 1]:
                    inv_d(m)
        dft16_pass(+1, st, after, [g for m in morder for g in range(NG) if GROUPS[g][0] == m])

    nb = S // tm

    def lanes(b, off=0, n=tm):
        st_ = b * tm + off
        return pl.ds(st_ if isinstance(st_, int) else pl.multiple_of(st_, 128), n)

    def ocp(b, i):
        hn = tm // nsp
        return pltpu.make_async_copy(o_v.at[b, :, pl.ds(i * hn, hn)], out_h.at[:, lanes(b, i * hn, hn)], osem.at[b, i])

    def p_vpu(b, t, prev, chain=chain, hs=0):
        h_v = h_l[hs]
        lh = slice(128 * t, 128 * t + 128)
        bx = min(b, nb - 1) if isinstance(b, int) else jnp.minimum(b, nb - 1)
        lx = lanes(bx, 128 * t, 128)
        lt = lx
        m1 = m1_v[:, lx]
        zf = pltpu.bitcast(tm_v[6, 0:8, :], F32)
        a2 = None
        for rg in range(64 // rows_):
            def rows(o):
                return slice(o + rows_ * rg, o + rows_ * rg + rows_)
            def bc(v):
                return v if rows_ == 8 else jnp.concatenate([v] * (rows_ // 8), axis=0)
            v0 = v_v[rows(0), lt] - bc(m1)
            if (chain & 1) and prev is not None:
                v0 = v0 + bc(prev * zf)
            vr = [v_v[rows(BLK_OFF[m]), lt] for m in (1, 2, 3)]
            vi = [v_v[rows(BLK_OFF[m] + 64), lt] for m in (1, 2, 3)]
            y = [None] * 7
            y[0] = v0 + (vr[0] + vr[1] + vr[2])
            for a in (1, 2, 3):
                A = _lin(vr, [_C7[(m * a) % 7] for m in (1, 2, 3)]) + v0
                B = _lin(vi, [_S7[(m * a) % 7] for m in (1, 2, 3)])
                y[a] = A - B
                y[7 - a] = A + B
            for a in range(7):
                hc = y[a] + x_v[rows(64 * a), lx].astype(F32)
                h_v[rows(64 * a), lh] = hc
                q = hc * hc
                if rows_ > 8:
                    q = sum(q[8 * i:8 * i + 8] for i in range(1, rows_ // 8)) + q[0:8]
                a2 = q if a2 is None else a2 + q
            prev = a2
        var = jnp.sum(a2, axis=0, keepdims=True) * (1.0 / D)
        r = jax.lax.rsqrt(var + 1e-5)
        ln = (h_v[:, lh] * r).astype(BF)
        lnp = pltpu.bitcast(ln.T, I32)
        ln_v[64 * t:64 * t + 64, :] = lnp
        return pltpu.bitcast(lnp[0:8, 0:128], F32) if (chain & 4) else a2

    def prep(b, chain=chain, hs=0):
        prev = None
        for t in range(tm // 128):
            prev = p_vpu(b, t, prev, chain, hs)

    def gate_up(c):
        cs = slice(c * fc, (c + 1) * fc)
        ln = _upk(ln_v[...])
        g = jnp.dot(ln, wg_v[:, cs], preferred_element_type=F32)
        u = jnp.dot(ln, wu_v[:, cs], preferred_element_type=F32)
        hh_v[:, cs] = _pk(g * u)

    ntt = tm // 128

    def down(b, hs=0):
        nt = (((1,), (1,)), ((), ()))
        hn = tm // nsp
        for i in range(nsp):
            o = jax.lax.dot_general(wd_v[...], _upk(hh_v[i * hn // 2:(i + 1) * hn // 2, :]), nt, preferred_element_type=F32)
            ls = lanes(b, i * hn, hn)
            o_v[b, :, i * hn:(i + 1) * hn] = ((h_l[hs][:, i * hn:(i + 1) * hn] + o) + m1_v[0:1, ls]).astype(BF)
            ocp(b, i).start()

    with sc('B0'):
        if wpos == 0:
            with sc('w_wg'):
                c_wg[0].wait()
            with sc('w_wu'):
                c_wu[0].wait()
        prep(0, 0)
        if wpos == 1:
            c_wg[0].wait()
            c_wu[0].wait()

    def block(b, first=False, last=False, hs=None, wdw=None):
        if hs is None:
            hs = b % 2
        for c in range(nfc):
            gate_up(c)
            if first and c == wdc:
                c_wd.wait()
            if wdw is not None and c == min(wdc, fsplit - 1):
                wdw()
        down(b, hs)
        if not last:
            prep(b + 1, chain, 1 - hs)

    def gu():
        for c in range(nfc):
            gate_up(c)

    if unroll == 9:
        c_wd.wait()
        o_v[0] = v_v[:, 0:tm].astype(BF)
        cpx = pltpu.make_async_copy(o_v.at[0], out_h.at[:, pl.ds(0, tm)], osem.at[0, 0])
        cpx.start()
        cpx.wait()
        return
    if unroll == 3:
        with sc('B1'):
            assert wdmid or fh == F
            if not wdmid:
                c_wd.wait()

            def late_wait(i):
                @pl.when(i == 0)
                def _():
                    for c in c_wgb + c_wub + [c_wd]:
                        c.wait()

            def body2(i, carry):
                block(2 * i, hs=0, wdw=(lambda: late_wait(i)) if wdmid else None)
                block(2 * i + 1, hs=1)
                return carry
            jax.lax.fori_loop(0, nb // 2, body2, 0)
    elif unroll == 4:
        with sc('B1'):
            pl.when(zero == 0)(gu)
            c_wd.wait()

            def body4(b, carry):
                down(b - 1)
                prep(b)
                gu()
                return carry
            jax.lax.fori_loop(1, nb, body4, 0)
            down(nb - 1)
    elif unroll == 5:
        with sc('B1'):
            block(0, first=True)
            pl.when(zero == 0)(lambda: None)
            jax.lax.fori_loop(1, nb, lambda b, c: (block(b), c)[1], 0)
    elif unroll:
        with sc('B1'):
            for b in range(nb):
                block(b, first=(b == 0), last=(b == nb - 1))
                if unroll == 2 and b < nb - 1:
                    pl.when(zero == 0)(lambda: None)
    else:
        with sc('B1'):
            if pbar:
                @pl.when(zero == 0)
                def _():
                    block(0, first=True)
            else:
                block(0, first=True)
        with sc('B2'):
            if peel_last:
                jax.lax.fori_loop(1, nb - 1, lambda b, c: (block(b), c)[1], 0)

                @pl.when(zero == 0)
                def _():
                    block(nb - 1, last=True)
            else:
                jax.lax.fori_loop(1, nb, lambda b, c: (block(b), c)[1], 0)
    for b in range(nb):
        for i in range(nsp):
            ocp(b, i).wait()


def make(tb=512, tm=512, fc=256, kw0=12, kw1=0, lag=4, scopes=False, bmode=1, nud=8, order=0, retile=True, flags=None, kc=256, wpos=1, dn=512, bar=1, unroll=3, tail=1, opq=3, tie=0, tlag=2, chain=5, nsp=2, pbar=1, peel_last=0, morder=(0, 1, 2, 3), rows_=8, wdc=6, wdmid=1, fsplit=7, xch=(4, 4, 4, 4), ra1=1):
    @jax.jit
    def f(A_x, A_w_r, A_w_i, B_x, B_w_gate, B_w_up, B_w_down):
        del B_x
        xT = A_x.reshape(S, D).T
        anyspec = pl.BlockSpec(memory_space=pl.ANY)
        scratch = [
            pltpu.VMEM((D, S), BF), pltpu.VMEM((H + 1, S), BF), pltpu.VMEM((H + 1, S), BF),
            pltpu.VMEM((D, F), BF), pltpu.VMEM((D, F), BF), pltpu.VMEM((D, F), BF),
            pltpu.VMEM((2, 32, 64), I32), pltpu.VMEM((7, 64, 128), I32), pltpu.VMEM((16, 64, 256), I32),
            pltpu.SMEM((1,), I32),
            [pltpu.VMEM((D // 2, S // nud), I32) for _ in range(nud)],
            pltpu.VMEM((8, S), F32), pltpu.VMEM((8, S), F32), pltpu.VMEM((D, S), F32), pltpu.VMEM((D // 2, S), I32),
            pltpu.VMEM((2, 16, H // 2, 128), I32),
            [pltpu.VMEM(((BLK_OFF[m + 1] - BLK_OFF[m]) // 2, S), I32) for m in range(4)], pltpu.VMEM((D, S), F32), [pltpu.VMEM((D, tm), F32) for _ in range(2)], pltpu.VMEM((tm // 2, D), I32),
            pltpu.VMEM((tm // 2, F), I32), pltpu.VMEM((S // tm, D, tm), BF),
            pltpu.SemaphoreType.DMA((len(xch) + 14,)), pltpu.SemaphoreType.DMA((S // tm, nsp)),
        ]
        outT = pl.pallas_call(
            functools.partial(_kernel, tb=tb, tm=tm, fc=fc, kw0=kw0, kw1=kw1, lag=lag, scopes=scopes, bmode=bmode, order=order, retile=retile, kc=kc, wpos=wpos, dn=dn, bar=bar, unroll=unroll, tail=tail, opq=opq, tie=tie, tlag=tlag, chain=chain, nsp=nsp, pbar=pbar, peel_last=peel_last, morder=morder, rows_=rows_, wdc=wdc, wdmid=wdmid, fsplit=fsplit, xch=xch, ra1=ra1),
            in_specs=[anyspec] * 10, out_specs=anyspec,
            out_shape=jax.ShapeDtypeStruct((D, S), BF),
            scratch_shapes=scratch,
            compiler_params=pltpu.CompilerParams(vmem_limit_bytes=100 * 1024 * 1024, flags=flags),
        )(xT, A_w_r.T, A_w_i.T, B_w_gate, B_w_up, B_w_down.T, _T0, _TM, _MM, np.zeros((1,), np.int32))
        return outT.T.reshape(1, S, D)
    return f


_fn = make(fsplit=4)


def pallas_sequential_preLN__spectral_gfnet__glu_gated_bilinear__prompt_kernel(A_x, A_w_r, A_w_i, B_x, B_w_gate, B_w_up, B_w_down):
    return _fn(A_x, A_w_r, A_w_i, B_x, B_w_gate, B_w_up, B_w_down)
```

```python
import contextlib
import functools
import numpy as np
import jax
import jax.numpy as jnp
from jax.experimental import pallas as pl
from jax.experimental.pallas import tpu as pltpu

S, D, F = 2048, 448, 1792
H = D // 2
NT = S // 128
NG = H // 8
EPS = 1e-5
BF = jnp.bfloat16
F32 = jnp.float32
I32 = jnp.int32

CLASSES = [[0, 7], [1, 8, 6, 13], [2, 9, 5, 12], [3, 10, 4, 11]]
GROUPS = [(m, kap, qh) for m in range(4) for kap in CLASSES[m] for qh in range(2)]
BLK = [0, 64, 192, 320, 448]
C7 = [float(np.cos(2 * np.pi * n / 7)) for n in range(7)]
S7 = [float(np.sin(2 * np.pi * n / 7)) for n in range(7)]
NT_DIMS = (((1,), (1,)), ((), ()))


def _np_packed(a):
    u = np.asarray(a, np.float32).astype(jnp.bfloat16.dtype).view(np.uint16).astype(np.uint32)
    return (u[..., 0::2, :] | (u[..., 1::2, :] << 16)).view(np.int32)


def _group_bins(g):
    _, kap, qh = GROUPS[g]
    j = 14 * (8 * qh + np.arange(8)) + kap
    return np.where(j == 0, H, j)


def _consts():
    b = np.arange(64)
    tf, ti = [], []
    for m in range(4):
        rows, cols = [], []
        for g in [g for g in range(NG) if GROUPS[g][0] == m]:
            j = _group_bins(g)
            th = 2 * np.pi * np.outer(j, b) / D
            c, s = np.cos(th), np.sin(th)
            if m == 0:
                fre, fim = c, np.where((j == H)[:, None], 0.0, -s)
                w = np.where(j == H, 1.0, 2.0)[:, None] / (S * D)
                ivr, ivi = (c * w).T, (fim * w).T
            else:
                sg = np.where((j % 7) == m, 1.0, -1.0)[:, None]

                def kord(p, q):
                    return np.stack([p.reshape(8, 4, 16), q.reshape(8, 4, 16)], axis=2).reshape(8, 128)
                fre, fim = kord(c, -sg * s), kord(-s, -sg * c)
                w = 2.0 / (S * D)
                ivr = np.concatenate([c * w, sg * s * w], 1).T
                ivi = np.concatenate([-s * w, sg * c * w], 1).T
            rows += [fre, fim]
            cols += [ivr, ivi]
        tf.append(np.concatenate(rows, 0))
        ti.append(np.concatenate(cols, 1))
    t0 = np.stack([tf[0], ti[0]])
    tm = np.stack(tf[1:] + ti[1:] + [np.zeros((128, 128))])
    v = np.arange(-16, 128)
    perm = 8 * (v % 16) + ((v // 16) % 8)
    s1 = np.arange(128)
    e = np.exp(-2j * np.pi * np.outer(perm, s1) / 128)
    t = np.exp(-2j * np.pi * np.outer(np.arange(16), s1) / S)
    et = np.concatenate([e.real, e.imag, t.real, t.imag], 0).astype(np.float32)
    return _np_packed(t0), _np_packed(tm), et


_T0, _TM, _ET = _consts()


def _pk(v):
    return pltpu.bitcast(v.astype(BF), I32)


def _upk(v):
    return pltpu.bitcast(v, BF)


def _dft4(a, sign):
    (r0, i0), (r1, i1), (r2, i2), (r3, i3) = a
    ar, ai = r0 + r2, i0 + i2
    br, bi = r0 - r2, i0 - i2
    cr, ci = r1 + r3, i1 + i3
    dr, di = r1 - r3, i1 - i3
    y0 = (ar + cr, ai + ci)
    y2 = (ar - cr, ai - ci)
    if sign < 0:
        y1 = (br + di, bi - dr)
        y3 = (br - di, bi + dr)
    else:
        y1 = (br - di, bi + dr)
        y3 = (br + di, bi - dr)
    return [y0, y1, y2, y3]


def _tw(v, n, sign):
    r, i = v
    if n == 0:
        return v
    if n == 4:
        return (i, -r) if sign < 0 else (-i, r)
    c = float(np.cos(2 * np.pi * n / 16))
    s = float(sign * np.sin(2 * np.pi * n / 16))
    if n % 2 == 0:
        same = (c * s) > 0
        return (((r - i) if same else (r + i)) * c, ((i + r) if same else (i - r)) * c)
    return (r * c - i * s, r * s + i * c)


def _dft16(v, sign, link=None):
    prev = None
    cols = []
    for n2 in range(4):
        a = [v[n2 + 4 * n1] for n1 in range(4)]
        if link is not None and prev is not None:
            a[0] = (link(a[0][0], prev), a[0][1])
        cols.append(_dft4(a, sign))
        prev = cols[-1][0][0]
    out = [None] * 16
    for k1 in range(4):
        a = [_tw(cols[n2][k1], n2 * k1, sign) for n2 in range(4)]
        if link is not None and k1 > 0:
            a[0] = (link(a[0][0], prev), a[0][1])
        y = _dft4(a, sign)
        prev = y[0][0]
        for k2 in range(4):
            out[k1 + 4 * k2] = y[k2]
    return out


def _lin(vals, coefs):
    acc = None
    for v, c in zip(vals, coefs):
        acc = v * c if acc is None else acc + v * c
    return acc


def _kernel(xT_h, wr_h, wi_h, wg_h, wu_h, wd_h, t0_h, tm_h, et_h, zs_h, out_h,
            x_v, wr_v, wi_v, wg_v, wu_v, wd_v, t0_v, tm_v, et_v, zs_s,
            mm_v, ud_l, r_v, m1_v, z_v, ws_v, yd_l, v_v, h_l, ln_v, hh_v, o_v, sem, osem,
            *, tm, fc, xch, fsplit, kwi, nsp, dn, a4link, plink, a3lag, scopes, a0pos, ra1, nearly, p0link, bars):
    sc = (lambda n: jax.named_scope(n)) if scopes else (lambda n: contextlib.nullcontext())
    nfc = F // fc
    nb = S // tm
    sems = iter(range(64))

    def copy(a, b):
        return pltpu.make_async_copy(a, b, sem.at[next(sems)])
    xo = [0]
    for n_ in xch:
        xo.append(xo[-1] + n_)
    assert xo[-1] == NT
    fh = fsplit * fc
    c_zs, c_et = copy(zs_h, zs_s), copy(et_h, et_v)
    c_x = [copy(xT_h.at[:, pl.ds(128 * xo[b], 128 * xch[b])], x_v.at[:, pl.ds(128 * xo[b], 128 * xch[b])])
           for b in range(len(xch))]
    c_t0, c_tm = copy(t0_h, t0_v), copy(tm_h, tm_v)
    c_wr, c_wi = copy(wr_h, wr_v), copy(wi_h, wi_v)
    c_wa = [copy(w_h.at[:, pl.ds(0, fh)], w_v.at[:, pl.ds(0, fh)]) for w_h, w_v in ((wg_h, wg_v), (wu_h, wu_v))]
    c_wb = [copy(w_h.at[:, pl.ds(fh, F - fh)], w_v.at[:, pl.ds(fh, F - fh)])
            for w_h, w_v in ((wg_h, wg_v), (wu_h, wu_v))] + [copy(wd_h, wd_v)]
    first = [c_zs, c_et, c_x[0]] if a0pos < 0 else [c_zs, c_x[0], c_et]
    for c in first + [c_t0, c_tm] + c_x[1:] + [c_wr, c_wi] + c_wa + c_wb:
        c.start()

    c_zs.wait()
    zero = zs_s[0]

    def phase(name):
        def deco(fn):
            with sc(name):
                if name in bars:
                    pl.when(zero == 0)(fn)
                else:
                    fn()
        return deco

    def ods(start, n):
        return pl.ds(pl.multiple_of(zero + start, 128), n)

    def gen_mats():
        c_et.wait()
        for k2 in range(16):
            er = et_v[16 - k2:144 - k2, :]
            ei = et_v[160 - k2:288 - k2, :]
            tr = et_v[288 + k2:289 + k2, :]
            ti = et_v[304 + k2:305 + k2, :]
            mr = er * tr - ei * ti
            mi = er * ti + ei * tr
            for a, val in enumerate((mr, mi, mr + mi)):
                mm_v[64 * a:64 * a + 64, 128 * k2:128 * k2 + 128] = _pk(val)

    def mmat(a, k2):
        return _upk(mm_v[64 * a:64 * a + 64, 128 * k2:128 * k2 + 128])

    def vpu_fwd(t):
        lo = 128 * t
        ud = ud_l[t % len(ud_l)]
        ul = slice(128 * (t // len(ud_l)), 128 * (t // len(ud_l)) + 128)
        u0s = []
        sq = None
        for bg in range(4):
            xa = [x_v[64 * a + 16 * bg:64 * a + 16 * bg + 16, lo:lo + 128].astype(F32) for a in range(7)]
            s_ = [xa[a] + xa[7 - a] for a in (1, 2, 3)]
            d_ = [xa[a] - xa[7 - a] for a in (1, 2, 3)]
            u0s.append(xa[0] + s_[0] + s_[1] + s_[2])
            for m in (1, 2, 3):
                ur = _lin(s_, [C7[(m * a) % 7] for a in (1, 2, 3)]) + xa[0]
                ui = _lin(d_, [S7[(m * a) % 7] for a in (1, 2, 3)])
                ud[64 * m - 32 + 16 * bg:64 * m - 24 + 16 * bg, ul] = _pk(ur)
                ud[64 * m - 24 + 16 * bg:64 * m - 16 + 16 * bg, ul] = _pk(ui)
                q = ur * ur + ui * ui
                sq = q if sq is None else sq + q
        m7 = jnp.sum(u0s[0] + u0s[1] + u0s[2] + u0s[3], axis=0, keepdims=True) * (1.0 / 64)
        sq = sq + sq
        for bg in range(4):
            uc = u0s[bg] - m7
            ud[8 * bg:8 * bg + 8, ul] = _pk(uc)
            sq = sq + uc * uc
        var = jnp.sum(sq, axis=0, keepdims=True) * (1.0 / (7 * D))
        r_v[:, lo:lo + 128] = jnp.broadcast_to(jax.lax.rsqrt(var + EPS), (8, 128))
        m1_v[:, lo:lo + 128] = jnp.broadcast_to(m7 * (1.0 / 7), (8, 128))

    def mxu_fwd(t):
        lo = 128 * t
        ud = ud_l[t % len(ud_l)]
        ul = ods(128 * (t // len(ud_l)), 128)
        r = r_v[0:1, lo:lo + 128] if ra1 else 1.0
        for m in range(4):
            tmat = _upk(t0_v[0]) if m == 0 else _upk(tm_v[m - 1])
            z_v[BLK[m]:BLK[m + 1], lo:lo + 128] = jnp.dot(
                tmat, _upk(ud[BLK[m] // 2:BLK[m + 1] // 2, ul]), preferred_element_type=F32) * r

    @phase('A1')
    def _():
        if a0pos < 0:
            gen_mats()
        for r_ in range(len(xch) + 1):
            if r_ < len(xch):
                c_x[r_].wait()
            if r_ == 1:
                c_t0.wait()
                c_tm.wait()
            if r_ > 0:
                for t in range(xo[r_ - 1], xo[r_]):
                    mxu_fwd(t)
            if r_ < len(xch):
                for t in range(xo[r_], xo[r_ + 1]):
                    vpu_fwd(t)
            if r_ == a0pos:
                gen_mats()

    zf_ = [None]

    def set_zf():
        zf_[0] = pltpu.bitcast(tm_v[6, 0:8, :], F32)

    def zlink(x, prev):
        return x + prev * zf_[0]

    def dft16_group(g, sign, link=None, prev=None):
        v = [(z_v[16 * g:16 * g + 8, 128 * t:128 * t + 128], z_v[16 * g + 8:16 * g + 16, 128 * t:128 * t + 128])
             for t in range(NT)]
        if sign < 0 and not ra1:
            v = [(a * r_v[:, 128 * t:128 * t + 128], b_ * r_v[:, 128 * t:128 * t + 128]) for t, (a, b_) in enumerate(v)]
        if prev is not None:
            v[0] = (zlink(v[0][0], prev), v[0][1])
        return _dft16(v, sign, link)

    @phase('A2')
    def _():
        for g in range(NG):
            o = dft16_group(g, -1)
            for t in range(NT):
                z_v[16 * g:16 * g + 8, 128 * t:128 * t + 128] = o[t][0]
                z_v[16 * g + 8:16 * g + 16, 128 * t:128 * t + 128] = o[t][1]


    def scramble(a, G):
        w_v = (wr_v, wi_v)[a]
        lane = jax.lax.broadcasted_iota(I32, (8, 128), 1)
        bits = [(lane & (1 << i)) != 0 for i in range(4)]
        cur = []
        for t in range(NT):
            blk = w_v[16 * G:16 * G + 16, 128 * t:128 * t + 128]
            if G == 0:
                row = jax.lax.broadcasted_iota(I32, (16, 128), 0)
                last = w_v[H:H + 1, 128 * t:128 * t + 128].astype(F32)
                blk = jnp.where(row == 0, last, blk.astype(F32)).astype(BF)
            v = pltpu.bitcast(blk, I32)
            cur.append(pltpu.roll(v, t, 1) if t else v)
        for i in range(4):
            cur = [jnp.where(bits[i], cur[(v + (1 << i)) % NT], cur[v]) for v in range(NT)]
        for k2 in range(NT):
            ws_v[a, k2, 8 * G:8 * G + 8, :] = cur[(-k2) % NT]

    def wload(a, k2):
        cls = [None] * 14
        for c in range(7):
            w = ws_v[a, k2, pl.ds(c, 16, stride=7), :]
            cls[2 * c] = pltpu.bitcast(w << 16, F32)
            cls[2 * c + 1] = pltpu.bitcast(w & jnp.int32(-65536), F32)
        return jnp.concatenate([cls[kap] for m in range(4) for kap in CLASSES[m]], axis=0).reshape(NG, 8, 128)

    def store_ri(k2, re, im):
        z_v[:, 128 * k2:128 * k2 + 128] = jnp.concatenate(
            [re.reshape(NG, 8, 128), im.reshape(NG, 8, 128)], axis=1).reshape(2 * H, 128)

    def load_ri(k2):
        xx = z_v[:, 128 * k2:128 * k2 + 128].reshape(NG, 16, 128)
        return xx[:, :8], xx[:, 8:]

    def flat(v):
        return v.reshape(H, 128).astype(BF)

    @phase('A3a')
    def _():
        todo = [[(0, G) for G in range(H // 16)], [(1, G) for G in range(H // 16)]]
        for k2 in range(16):
            if k2 == 0:
                c_wr.wait()
            if k2 == kwi:
                c_wi.wait()
            ur, ui = load_ri(k2)
            t1 = jax.lax.dot_general(flat(ur), mmat(0, k2), NT_DIMS, preferred_element_type=F32)
            t2 = jax.lax.dot_general(flat(ui), mmat(1, k2), NT_DIMS, preferred_element_type=F32)
            t3 = jax.lax.dot_general(flat(ur + ui), mmat(2, k2), NT_DIMS, preferred_element_type=F32)
            store_ri(k2, t1 - t2, (t3 - t1) - t2)
            seg, end = (0, kwi) if k2 < kwi else (1, 16)
            for _ in range(-(-len(todo[seg]) // (end - k2))):
                scramble(*todo[seg].pop(0))

    @phase('A3b')
    def _():
        for k2 in range(16):
            xr, xi = load_ri(k2)
            wr, wi = wload(0, k2), wload(1, k2)
            vr = xr * wr - xi * wi
            vi = xr * wi + xi * wr
            t1 = jnp.dot(flat(vr), mmat(0, k2), preferred_element_type=F32)
            t2 = jnp.dot(flat(vi), mmat(1, k2), preferred_element_type=F32)
            t3 = jnp.dot(flat(vi - vr), mmat(2, k2), preferred_element_type=F32)
            store_ri(k2, t1 + t2, (t3 + t1) - t2)

    def inv_dot(m, c):
        tmat = _upk(t0_v[1]) if m == 0 else _upk(tm_v[2 + m])
        v_v[BLK[m]:BLK[m + 1], c * dn:(c + 1) * dn] = jnp.dot(
            tmat, _upk(yd_l[m][:, ods(c * dn, dn)]), preferred_element_type=F32)

    @phase('A4')
    def _():
        set_zf()
        prev = None
        for g in range(NG):
            m = GROUPS[g][0]
            gg = g - BLK[m] // 16
            o = dft16_group(g, +1, zlink if a4link >= 2 else None, prev if a4link >= 1 else None)
            prev = o[0][0]
            for t in range(NT):
                yd_l[m][8 * gg:8 * gg + 8, 128 * t:128 * t + 128] = _pk(jnp.concatenate(o[t], axis=0))
            if 16 * (g + 1) == BLK[m + 1]:
                for c in range(nearly):
                    inv_dot(m, c)

    def lanes(b, off, n):
        st_ = b * tm + off
        return pl.ds(st_ if isinstance(st_, int) else pl.multiple_of(st_, 128), n)

    def prep_tile(b, t, hs, prev, link):
        h_v = h_l[hs]
        lh = slice(128 * t, 128 * t + 128)
        bx = min(b, nb - 1) if isinstance(b, int) else jnp.minimum(b, nb - 1)
        lx = lanes(bx, 128 * t, 128)
        m1 = m1_v[:, lx]
        a2 = None
        for rg in range(8):
            def rows(o):
                return slice(o + 8 * rg, o + 8 * rg + 8)
            v0 = v_v[rows(0), lx] - m1
            if link and prev is not None:
                v0 = zlink(v0, prev)
            vr = [v_v[rows(BLK[m]), lx] for m in (1, 2, 3)]
            vi = [v_v[rows(BLK[m] + 64), lx] for m in (1, 2, 3)]
            y = [None] * 7
            y[0] = v0 + (vr[0] + vr[1] + vr[2])
            for a in (1, 2, 3):
                A = _lin(vr, [C7[(m * a) % 7] for m in (1, 2, 3)]) + v0
                B = _lin(vi, [S7[(m * a) % 7] for m in (1, 2, 3)])
                y[a] = A - B
                y[7 - a] = A + B
            for a in range(7):
                hc = y[a] + x_v[rows(64 * a), lx].astype(F32)
                h_v[rows(64 * a), lh] = hc
                a2 = hc * hc if a2 is None else a2 + hc * hc
            prev = a2
        var = jnp.sum(a2, axis=0, keepdims=True) * (1.0 / D)
        r = jax.lax.rsqrt(var + EPS)
        lnp = pltpu.bitcast((h_v[:, lh] * r).astype(BF).T, I32)
        ln_v[64 * t:64 * t + 64, :] = lnp
        return pltpu.bitcast(lnp[0:8, 0:128], F32) if link >= 2 else a2

    def prep(b, hs, link):
        prev = None
        for t in range(tm // 128):
            prev = prep_tile(b, t, hs, prev, link)

    hn = tm // nsp

    def ocp(b, i):
        return pltpu.make_async_copy(o_v.at[b, :, pl.ds(i * hn, hn)], out_h.at[:, lanes(b, i * hn, hn)], osem.at[b, i])

    def block(b, hs, late_wait=None):
        for c in range(nfc):
            cs = slice(c * fc, (c + 1) * fc)
            ln = _upk(ln_v[...])
            g = jnp.dot(ln, wg_v[:, cs], preferred_element_type=F32)
            u = jnp.dot(ln, wu_v[:, cs], preferred_element_type=F32)
            hh_v[:, cs] = _pk(g * u)
            if late_wait is not None and c == fsplit - 1:
                late_wait()
        for i in range(nsp):
            o = jax.lax.dot_general(wd_v[...], _upk(hh_v[i * hn // 2:(i + 1) * hn // 2, :]), NT_DIMS,
                                    preferred_element_type=F32)
            ls = lanes(b, i * hn, hn)
            o_v[b, :, i * hn:(i + 1) * hn] = ((h_l[hs][:, i * hn:(i + 1) * hn] + o) + m1_v[0:1, ls]).astype(BF)
            ocp(b, i).start()
        prep(b + 1, 1 - hs, plink)

    @phase('B0')
    def _():
        set_zf()
        for c in range(nearly, S // dn):
            for m in range(4):
                inv_dot(m, c)
        prep(0, 0, p0link)
        for c in c_wa:
            c.wait()

    with sc('B1'):
        set_zf()
        def body(i, carry):
            def late_wait():
                @pl.when(i == 0)
                def _():
                    for c in c_wb:
                        c.wait()
            block(2 * i, 0, late_wait)
            block(2 * i + 1, 1)
            return carry
        jax.lax.fori_loop(0, nb // 2, body, 0)
    for b in range(nb):
        for i in range(nsp):
            ocp(b, i).wait()


def make(tm=512, fc=256, xch=(4, 4, 4, 2, 2), fsplit=4, kwi=8, nsp=2, dn=512, a4link=0, plink=2, a3lag=0,
         nud=8, scopes=False, a0pos=0, ra1=0, nearly=1, p0link=1, bars=('A4',)):
    @jax.jit
    def f(A_x, A_w_r, A_w_i, B_x, B_w_gate, B_w_up, B_w_down):
        del B_x
        anyspec = pl.BlockSpec(memory_space=pl.ANY)
        scratch = [
            pltpu.VMEM((D, S), BF), pltpu.VMEM((H + 1, S), BF), pltpu.VMEM((H + 1, S), BF),
            pltpu.VMEM((D, F), BF), pltpu.VMEM((D, F), BF), pltpu.VMEM((D, F), BF),
            pltpu.VMEM((2, 32, 64), I32), pltpu.VMEM((7, 64, 128), I32), pltpu.VMEM((320, 128), F32),
            pltpu.SMEM((1,), I32),
            pltpu.VMEM((192, S), I32),
            [pltpu.VMEM((D // 2, S // nud), I32) for _ in range(nud)],
            pltpu.VMEM((8, S), F32), pltpu.VMEM((8, S), F32), pltpu.VMEM((D, S), F32),
            pltpu.VMEM((2, 16, H // 2, 128), I32),
            [pltpu.VMEM(((BLK[m + 1] - BLK[m]) // 2, S), I32) for m in range(4)],
            pltpu.VMEM((D, S), F32), [pltpu.VMEM((D, tm), F32) for _ in range(2)],
            pltpu.VMEM((tm // 2, D), I32), pltpu.VMEM((tm // 2, F), I32),
            pltpu.VMEM((S // tm, D, tm), BF),
            pltpu.SemaphoreType.DMA((len(xch) + 12,)), pltpu.SemaphoreType.DMA((S // tm, nsp)),
        ]
        outT = pl.pallas_call(
            functools.partial(_kernel, tm=tm, fc=fc, xch=xch, fsplit=fsplit, kwi=kwi, nsp=nsp, dn=dn,
                              a4link=a4link, plink=plink, a3lag=a3lag, scopes=scopes, a0pos=a0pos, ra1=ra1, nearly=nearly, p0link=p0link, bars=bars),
            in_specs=[anyspec] * 10, out_specs=anyspec,
            out_shape=jax.ShapeDtypeStruct((D, S), BF),
            scratch_shapes=scratch,
            compiler_params=pltpu.CompilerParams(vmem_limit_bytes=100 * 1024 * 1024),
        )(A_x.reshape(S, D).T, A_w_r.T, A_w_i.T, B_w_gate, B_w_up, B_w_down.T, _T0, _TM, _ET,
          np.zeros((1,), np.int32))
        return outT.T.reshape(1, S, D)
    return f


_fn = make()


def pallas_sequential_preLN__spectral_gfnet__glu_gated_bilinear__prompt_kernel(A_x, A_w_r, A_w_i, B_x, B_w_gate, B_w_up, B_w_down):
    return _fn(A_x, A_w_r, A_w_i, B_x, B_w_gate, B_w_up, B_w_down)
```

```python
import numpy as np
import jax
import jax.numpy as jnp
import jax.experimental.pallas as pl
import jax.experimental.pallas.tpu as pltpu

S, D, F = 2048, 448, 1792
H = D // 2
NT = S // 128
NG = H // 8
EPS = 1e-5
TM = 512
NB = S // TM
FC = 256
XCH = (4, 4, 4, 2, 2)
NSP = (1, 4)
KWI = 8
NUD = 8
BF, F32, I32 = jnp.bfloat16, jnp.float32, jnp.int32
NT_DIMS = (((1,), (1,)), ((), ()))

CLASSES = [[0, 7], [1, 8, 6, 13], [2, 9, 5, 12], [3, 10, 4, 11]]
GROUPS = [(m, kap, qh) for m in range(4) for kap in CLASSES[m] for qh in range(2)]
BLK = [0, 64, 192, 320, 448]
C7 = [float(np.cos(2 * np.pi * n / 7)) for n in range(7)]
S7 = [float(np.sin(2 * np.pi * n / 7)) for n in range(7)]


def _np_packed(a):
    u = np.asarray(a, np.float32).astype(jnp.bfloat16.dtype).view(np.uint16).astype(np.uint32)
    return (u[..., 0::2, :] | (u[..., 1::2, :] << 16)).view(np.int32)


def _consts():
    b = np.arange(64)
    tf, ti = [], []
    for m in range(4):
        rows, cols = [], []
        for mm, kap, qh in GROUPS:
            if mm != m:
                continue
            j = 14 * (8 * qh + np.arange(8)) + kap
            j = np.where(j == 0, H, j)
            th = 2 * np.pi * np.outer(j, b) / D
            c, s = np.cos(th), np.sin(th)
            if m == 0:
                fre, fim = c, np.where((j == H)[:, None], 0.0, -s)
                w = np.where(j == H, 1.0, 2.0)[:, None] / (S * D)
                ivr, ivi = (c * w).T, (fim * w).T
            else:
                sg = np.where((j % 7) == m, 1.0, -1.0)[:, None]

                def kord(p, q):
                    return np.stack([p.reshape(8, 4, 16), q.reshape(8, 4, 16)], axis=2).reshape(8, 128)
                fre, fim = kord(c, -sg * s), kord(-s, -sg * c)
                w = 2.0 / (S * D)
                ivr = np.concatenate([c * w, sg * s * w], 1).T
                ivi = np.concatenate([-s * w, sg * c * w], 1).T
            rows += [fre, fim]
            cols += [ivr, ivi]
        tf.append(np.concatenate(rows, 0))
        ti.append(np.concatenate(cols, 1))
    t0 = np.stack([tf[0], ti[0]])
    tm = np.stack(tf[1:] + ti[1:] + [np.zeros((128, 128))])
    v = np.arange(-16, 128)
    perm = 8 * (v % 16) + ((v // 16) % 8)
    s1 = np.arange(128)
    e = np.exp(-2j * np.pi * np.outer(perm, s1) / 128)
    t = np.exp(-2j * np.pi * np.outer(np.arange(16), s1) / S)
    et = np.concatenate([e.real, e.imag, t.real, t.imag], 0).astype(np.float32)
    return _np_packed(t0), _np_packed(tm), et


_T0, _TM, _ET = _consts()


def _pk(v):
    return pltpu.bitcast(v.astype(BF), I32)


def _upk(v):
    return pltpu.bitcast(v, BF)


def _dft4(a, sign):
    (r0, i0), (r1, i1), (r2, i2), (r3, i3) = a
    ar, ai = r0 + r2, i0 + i2
    br, bi = r0 - r2, i0 - i2
    cr, ci = r1 + r3, i1 + i3
    dr, di = r1 - r3, i1 - i3
    y1, y3 = (br + di, bi - dr), (br - di, bi + dr)
    if sign > 0:
        y1, y3 = y3, y1
    return [(ar + cr, ai + ci), y1, (ar - cr, ai - ci), y3]


def _tw(v, n, sign):
    r, i = v
    if n == 0:
        return v
    if n == 4:
        return (i, -r) if sign < 0 else (-i, r)
    c = float(np.cos(2 * np.pi * n / 16))
    s = float(sign * np.sin(2 * np.pi * n / 16))
    if n % 2 == 0:
        same = (c * s) > 0
        return (((r - i) if same else (r + i)) * c, ((i + r) if same else (i - r)) * c)
    return (r * c - i * s, r * s + i * c)


def _dft16(v, sign):
    cols = [_dft4([v[n2 + 4 * n1] for n1 in range(4)], sign) for n2 in range(4)]
    out = [None] * 16
    for k1 in range(4):
        y = _dft4([_tw(cols[n2][k1], n2 * k1, sign) for n2 in range(4)], sign)
        for k2 in range(4):
            out[k1 + 4 * k2] = y[k2]
    return out


def _lin(vals, coefs):
    acc = None
    for v, c in zip(vals, coefs):
        acc = v * c if acc is None else acc + v * c
    return acc


def _kernel(xT_h, wr_h, wi_h, wg_h, wu_h, wd_h, t0_h, tm_h, et_h, zs_h, out_h,
            x_v, wr_v, wi_v, wg_v, wu_v, wd_v, t0_v, tm_v, et_v, zs_s,
            mm_v, ud_l, r_v, m1_v, z_v, ws_v, yd_l, v_v, h_l, ln_v, hh_v, o_v, sem, osem):
    sems = iter(range(len(XCH) + 11))

    def copy(a, b):
        return pltpu.make_async_copy(a, b, sem.at[next(sems)])

    xo = [int(n) for n in np.cumsum((0,) + XCH)]
    c_zs, c_et, c_t0 = copy(zs_h, zs_s), copy(et_h, et_v), copy(t0_h, t0_v)
    c_x = [copy(xT_h.at[:, pl.ds(128 * xo[c], 128 * XCH[c])], x_v.at[:, pl.ds(128 * xo[c], 128 * XCH[c])])
           for c in range(len(XCH))]
    c_tf = copy(tm_h.at[pl.ds(0, 3)], tm_v.at[pl.ds(0, 3)])
    c_ti = copy(tm_h.at[pl.ds(3, 4)], tm_v.at[pl.ds(3, 4)])
    c_wr, c_wi = copy(wr_h, wr_v), copy(wi_h, wi_v)
    c_wg, c_wu, c_wd = copy(wg_h, wg_v), copy(wu_h, wu_v), copy(wd_h, wd_v)
    for c in [c_zs, c_x[0], c_et, c_t0, c_tf] + c_x[1:] + [c_wr, c_wi, c_ti, c_wg, c_wu, c_wd]:
        c.start()

    c_zs.wait()
    zero = zs_s[0]

    def ods(start, n):
        return pl.ds(pl.multiple_of(zero + start, 128), n)

    def tile(t):
        return slice(128 * t, 128 * t + 128)

    def gen_mats():
        c_et.wait()
        for k2 in range(NT):
            er, ei = et_v[16 - k2:144 - k2, :], et_v[160 - k2:288 - k2, :]
            tr, ti = et_v[288 + k2:289 + k2, :], et_v[304 + k2:305 + k2, :]
            mr = er * tr - ei * ti
            mi = er * ti + ei * tr
            for a, val in enumerate((mr, mi, mr + mi)):
                mm_v[64 * a:64 * a + 64, tile(k2)] = _pk(val)

    def mmat(a, k2):
        return _upk(mm_v[64 * a:64 * a + 64, tile(k2)])

    def vpu_fwd(t):
        ud, ul = ud_l[t % NUD], tile(t // NUD)
        u0s, sq = [], None
        for bg in range(4):
            xa = [x_v[64 * a + 16 * bg:64 * a + 16 * bg + 16, tile(t)].astype(F32) for a in range(7)]
            s_ = [xa[a] + xa[7 - a] for a in (1, 2, 3)]
            d_ = [xa[a] - xa[7 - a] for a in (1, 2, 3)]
            u0s.append(xa[0] + s_[0] + s_[1] + s_[2])
            for m in (1, 2, 3):
                ur = _lin(s_, [C7[(m * a) % 7] for a in (1, 2, 3)]) + xa[0]
                ui = _lin(d_, [S7[(m * a) % 7] for a in (1, 2, 3)])
                o = BLK[m] // 2 + 16 * bg
                ud[o:o + 8, ul] = _pk(ur)
                ud[o + 8:o + 16, ul] = _pk(ui)
                q = ur * ur + ui * ui
                sq = q if sq is None else sq + q
        m7 = jnp.sum(u0s[0] + u0s[1] + u0s[2] + u0s[3], axis=0, keepdims=True) * (1.0 / 64)
        sq = sq + sq
        for bg in range(4):
            uc = u0s[bg] - m7
            ud[8 * bg:8 * bg + 8, ul] = _pk(uc)
            sq = sq + uc * uc
        var = jnp.sum(sq, axis=0, keepdims=True) * (1.0 / (7 * D))
        r_v[:, tile(t)] = jnp.broadcast_to(jax.lax.rsqrt(var + EPS), (8, 128))
        m1_v[:, tile(t)] = jnp.broadcast_to(m7 * (1.0 / 7), (8, 128))

    def mxu_fwd(t):
        ud, ul = ud_l[t % NUD], ods(128 * (t // NUD), 128)
        for m in range(4):
            tmat = _upk(t0_v[0]) if m == 0 else _upk(tm_v[m - 1])
            z_v[BLK[m]:BLK[m + 1], tile(t)] = jnp.dot(
                tmat, _upk(ud[BLK[m] // 2:BLK[m + 1] // 2, ul]), preferred_element_type=F32)

    for c in range(len(XCH) + 1):
        if c < len(XCH):
            c_x[c].wait()
        if c == 1:
            c_t0.wait()
            c_tf.wait()
        if c > 0:
            for t in range(xo[c - 1], xo[c]):
                mxu_fwd(t)
        if c < len(XCH):
            for t in range(xo[c], xo[c + 1]):
                vpu_fwd(t)
        if c == 0:
            gen_mats()

    def group(g):
        return [(z_v[16 * g:16 * g + 8, tile(t)], z_v[16 * g + 8:16 * g + 16, tile(t)]) for t in range(NT)]

    for g in range(NG):
        o = _dft16([(a * r_v[:, tile(t)], b * r_v[:, tile(t)]) for t, (a, b) in enumerate(group(g))], -1)
        for t in range(NT):
            z_v[16 * g:16 * g + 8, tile(t)] = o[t][0]
            z_v[16 * g + 8:16 * g + 16, tile(t)] = o[t][1]

    def scramble(a, G):
        w_v = (wr_v, wi_v)[a]
        lane = jax.lax.broadcasted_iota(I32, (8, 128), 1)
        cur = []
        for t in range(NT):
            blk = w_v[16 * G:16 * G + 16, tile(t)]
            if G == 0:
                row = jax.lax.broadcasted_iota(I32, (16, 128), 0)
                blk = jnp.where(row == 0, w_v[H:H + 1, tile(t)].astype(F32), blk.astype(F32)).astype(BF)
            v = pltpu.bitcast(blk, I32)
            cur.append(pltpu.roll(v, t, 1) if t else v)
        for i in range(4):
            bit = (lane & (1 << i)) != 0
            cur = [jnp.where(bit, cur[(v + (1 << i)) % NT], cur[v]) for v in range(NT)]
        for k2 in range(NT):
            ws_v[a, k2, 8 * G:8 * G + 8, :] = cur[(-k2) % NT]

    def wload(a, k2):
        cls = [None] * 14
        for c in range(7):
            w = ws_v[a, k2, pl.ds(c, 16, stride=7), :]
            cls[2 * c] = pltpu.bitcast(w << 16, F32)
            cls[2 * c + 1] = pltpu.bitcast(w & np.int32(-65536), F32)
        return jnp.concatenate([cls[kap] for m in range(4) for kap in CLASSES[m]], axis=0).reshape(NG, 8, 128)

    def load_ri(k2):
        xx = z_v[:, tile(k2)].reshape(NG, 16, 128)
        return xx[:, :8], xx[:, 8:]

    def store_ri(k2, re, im):
        z_v[:, tile(k2)] = jnp.concatenate(
            [re.reshape(NG, 8, 128), im.reshape(NG, 8, 128)], axis=1).reshape(2 * H, 128)

    def flat(v):
        return v.reshape(H, 128).astype(BF)

    todo = [list(range(H // 16)), list(range(H // 16))]
    for k2 in range(NT):
        if k2 == 0:
            c_wr.wait()
        if k2 == KWI:
            c_wi.wait()
        ur, ui = load_ri(k2)
        t1 = jax.lax.dot_general(flat(ur), mmat(0, k2), NT_DIMS, preferred_element_type=F32)
        t2 = jax.lax.dot_general(flat(ui), mmat(1, k2), NT_DIMS, preferred_element_type=F32)
        t3 = jax.lax.dot_general(flat(ur + ui), mmat(2, k2), NT_DIMS, preferred_element_type=F32)
        store_ri(k2, t1 - t2, (t3 - t1) - t2)
        a, end = (0, KWI) if k2 < KWI else (1, NT)
        for _ in range(-(-len(todo[a]) // (end - k2))):
            scramble(a, todo[a].pop(0))

    for k2 in range(NT):
        xr, xi = load_ri(k2)
        wr, wi = wload(0, k2), wload(1, k2)
        vr = xr * wr - xi * wi
        vi = xr * wi + xi * wr
        t1 = jnp.dot(flat(vr), mmat(0, k2), preferred_element_type=F32)
        t2 = jnp.dot(flat(vi), mmat(1, k2), preferred_element_type=F32)
        t3 = jnp.dot(flat(vi - vr), mmat(2, k2), preferred_element_type=F32)
        store_ri(k2, t1 + t2, (t3 + t1) - t2)

    def inv_dot(m, b):
        tmat = _upk(t0_v[1]) if m == 0 else _upk(tm_v[2 + m])
        v_v[BLK[m]:BLK[m + 1], b * TM:(b + 1) * TM] = jnp.dot(
            tmat, _upk(yd_l[m][:, ods(b * TM, TM)]), preferred_element_type=F32)

    @pl.when(zero == 0)
    def _():
        c_ti.wait()
        for g in range(NG):
            m = GROUPS[g][0]
            gg = g - BLK[m] // 16
            o = _dft16(group(g), +1)
            for t in range(NT):
                yd_l[m][8 * gg:8 * gg + 8, tile(t)] = _pk(jnp.concatenate(o[t], axis=0))
            if 16 * (g + 1) == BLK[m + 1]:
                inv_dot(m, 0)

    def lanes(b, off, n):
        st = b * TM + off
        return pl.ds(st if isinstance(st, int) else pl.multiple_of(st, 128), n)

    def prep(b, hs, link):
        zvec = tm_v[6, 0:8, :]
        bx = min(b, NB - 1) if isinstance(b, int) else jnp.minimum(b, NB - 1)
        h_v, prev = h_l[hs], None
        for t in range(TM // 128):
            lx = lanes(bx, 128 * t, 128)
            m1 = m1_v[:, lx]
            a2 = None
            for rg in range(8):
                def rows(o):
                    return slice(o + 8 * rg, o + 8 * rg + 8)
                v0 = v_v[rows(0), lx] - m1
                if prev is not None:
                    v0 = v0 + pltpu.bitcast(pltpu.bitcast(prev, I32) & zvec, F32)
                vr = [v_v[rows(BLK[m]), lx] for m in (1, 2, 3)]
                vi = [v_v[rows(BLK[m] + 64), lx] for m in (1, 2, 3)]
                y = [None] * 7
                y[0] = v0 + (vr[0] + vr[1] + vr[2])
                for a in (1, 2, 3):
                    ca = _lin(vr, [C7[(m * a) % 7] for m in (1, 2, 3)]) + v0
                    sa = _lin(vi, [S7[(m * a) % 7] for m in (1, 2, 3)])
                    y[a], y[7 - a] = ca - sa, ca + sa
                for a in range(7):
                    hc = y[a] + x_v[rows(64 * a), lx].astype(F32)
                    h_v[rows(64 * a), tile(t)] = hc
                    a2 = hc * hc if a2 is None else a2 + hc * hc
                prev = a2
            var = jnp.sum(a2, axis=0, keepdims=True) * (1.0 / D)
            lnp = pltpu.bitcast((h_v[:, tile(t)] * jax.lax.rsqrt(var + EPS)).astype(BF).T, I32)
            ln_v[64 * t:64 * t + 64, :] = lnp
            if link:
                prev = pltpu.bitcast(lnp[0:8, 0:128], F32)

    def ocp(b, i, hs):
        hn = TM // NSP[hs]
        return pltpu.make_async_copy(o_v.at[b, :, pl.ds(i * hn, hn)], out_h.at[:, lanes(b, i * hn, hn)],
                                     osem.at[b * max(NSP) + i])

    def block(b, hs, late_wait=None):
        for c in range(F // FC):
            cs = slice(c * FC, (c + 1) * FC)
            ln = _upk(ln_v[...])
            g = jnp.dot(ln, wg_v[:, cs], preferred_element_type=F32)
            u = jnp.dot(ln, wu_v[:, cs], preferred_element_type=F32)
            hh_v[:, cs] = _pk(g * u)
        if late_wait is not None:
            late_wait()
        hn = TM // NSP[hs]
        for i in range(NSP[hs]):
            o = jax.lax.dot_general(wd_v[...], _upk(hh_v[i * hn // 2:(i + 1) * hn // 2, :]), NT_DIMS,
                                    preferred_element_type=F32)
            o_v[b, :, i * hn:(i + 1) * hn] = (
                (h_l[hs][:, i * hn:(i + 1) * hn] + o) + m1_v[0:1, lanes(b, i * hn, hn)]).astype(BF)
            ocp(b, i, hs).start()
        prep(b + 1, 1 - hs, True)

    for b in range(1, NB):
        for m in range(4):
            inv_dot(m, b)
    prep(0, 0, False)
    c_wg.wait()
    c_wu.wait()

    def body(i, carry):
        def late_wait():
            @pl.when(i == 0)
            def _():
                c_wd.wait()
        block(2 * i, 0, late_wait)
        block(2 * i + 1, 1)
        return carry

    jax.lax.fori_loop(0, NB // 2, body, 0)
    for b in range(NB):
        for i in range(NSP[b % 2]):
            ocp(b, i, b % 2).wait()


@jax.jit
def pallas_sequential_preLN__spectral_gfnet__glu_gated_bilinear__prompt_kernel(
    A_x: jax.Array,
    A_w_r: jax.Array,
    A_w_i: jax.Array,
    B_x: jax.Array,
    B_w_gate: jax.Array,
    B_w_up: jax.Array,
    B_w_down: jax.Array,
):
    del B_x
    hbm = pl.BlockSpec(memory_space=pl.ANY)
    scratch = [
        pltpu.VMEM((D, S), BF),
        pltpu.VMEM((H + 1, S), BF), pltpu.VMEM((H + 1, S), BF),
        pltpu.VMEM((D, F), BF), pltpu.VMEM((D, F), BF), pltpu.VMEM((D, F), BF),
        pltpu.VMEM((2, 32, 64), I32), pltpu.VMEM((7, 64, 128), I32),
        pltpu.VMEM((320, 128), F32), pltpu.SMEM((1,), I32),
        pltpu.VMEM((192, S), I32),
        [pltpu.VMEM((D // 2, S // NUD), I32) for _ in range(NUD)],
        pltpu.VMEM((8, S), F32), pltpu.VMEM((8, S), F32),
        pltpu.VMEM((D, S), F32),
        pltpu.VMEM((2, NT, H // 2, 128), I32),
        [pltpu.VMEM(((BLK[m + 1] - BLK[m]) // 2, S), I32) for m in range(4)],
        pltpu.VMEM((D, S), F32),
        [pltpu.VMEM((D, TM), F32) for _ in range(2)],
        pltpu.VMEM((TM // 2, D), I32), pltpu.VMEM((TM // 2, F), I32),
        pltpu.VMEM((NB, D, TM), BF),
        pltpu.SemaphoreType.DMA((len(XCH) + 11,)), pltpu.SemaphoreType.DMA((NB * max(NSP),)),
    ]
    out_t = pl.pallas_call(
        _kernel,
        in_specs=[hbm] * 10,
        out_specs=hbm,
        out_shape=jax.ShapeDtypeStruct((D, S), BF),
        scratch_shapes=scratch,
        compiler_params=pltpu.CompilerParams(vmem_limit_bytes=64 * 1024 * 1024),
    )(A_x.reshape(S, D).T, A_w_r.T, A_w_i.T, B_w_gate, B_w_up, B_w_down.T,
      _T0, _TM, _ET, np.zeros((1,), np.int32))
    return out_t.T.reshape(1, S, D)
```
